```python
import jax
import jax.numpy as jnp

def _softmax(x, axis=-1):
    return jax.nn.softmax(x, axis=axis)
def _gelu(x):
    return jax.nn.gelu(x, approximate=True)
def _silu(x):
    return jax.nn.silu(x)
def _sigmoid(x):
    return jax.nn.sigmoid(x)
def _layernorm(x, axis=-1, eps=1e-5):
    m = jnp.mean(x, axis=axis, keepdims=True)
    v = jnp.var(x, axis=axis, keepdims=True)
    return (x - m) / jnp.sqrt(v + eps)
def _scatter_add(tgt, idx, src, axis=0):
    return tgt.at[idx].add(src)
def _segment_sum(src, seg, n):
    return jax.ops.segment_sum(src, seg, n)
class _Rng:
    def __init__(self, key):
        self._k = key
    def _next(self):
        self._k, sub = jax.random.split(self._k)
        return sub
    def normal(self, shape):
        return jax.random.normal(self._next(), shape, dtype=jnp.bfloat16)
    def randint(self, lo, hi, shape):
        return jax.random.randint(self._next(), shape, lo, hi, dtype=jnp.int32)
    def uniform(self, shape, lo=0.0, hi=1.0):
        return jax.random.uniform(self._next(), shape, jnp.bfloat16, lo, hi)
    def permutation(self, n):
        return jax.random.permutation(self._next(), n)


kernel_name = 'gated_mix__mha_block_cached__moe_arch_mod__decode'

def setup_inputs():
    _rng = _Rng(jax.random.key(int.from_bytes(__import__("os").urandom(4), "little")))
    _w = (lambda a: (lambda t: t.astype(jnp.bfloat16) if jnp.issubdtype(t.dtype, jnp.floating) else t)(jnp.asarray(a)))
    def _A_setup():
        B, Sq, D = 4, 1, 1024
        H, Sk, Dh = 32, 8192, 128
        return {
            "x": _w((lambda *s: _rng.normal(s) * 0.05)(B, Sq, D)),
            "k_cache": _w((lambda *s: _rng.normal(s) * 0.05)(B, H, Sk, Dh)),
            "v_cache": _w((lambda *s: _rng.normal(s) * 0.05)(B, H, Sk, Dh)),
            "wq": _w((lambda *s: _rng.normal(s) * 0.05)(D, H * Dh) * (D ** -0.5)),
            "wo": _w((lambda *s: _rng.normal(s) * 0.05)(H * Dh, D) * ((H * Dh) ** -0.5)),
        }
    _A_in = _A_setup()

    def _B_setup():
        B, S, D, F, C = 4, 1, 1024, 3584, 1
        return {
            "x": _w((lambda *s: _rng.normal(s) * 0.05)(B, S, D)),
            "w_r": _w((lambda *s: _rng.normal(s) * 0.05)(D)),
            "w_gate": _w((lambda *s: _rng.normal(s) * 0.05)(D, F)),
            "w_up": _w((lambda *s: _rng.normal(s) * 0.05)(D, F)),
            "w_down": _w((lambda *s: _rng.normal(s) * 0.05)(F, D)),
        }
    _B_in = _B_setup()

    return {
        "A_x": _A_in["x"],
        "A_k_cache": _A_in["k_cache"],
        "A_v_cache": _A_in["v_cache"],
        "A_wq": _A_in["wq"],
        "A_wo": _A_in["wo"],
        "B_x": _B_in["x"],
        "B_w_r": _B_in["w_r"],
        "B_w_gate": _B_in["w_gate"],
        "B_w_up": _B_in["w_up"],
        "B_w_down": _B_in["w_down"],
        "gate_w": _w((lambda *s: _rng.normal(s) * 0.05)(1024)),
    }

def reference(A_x, A_k_cache, A_v_cache, A_wq, A_wo, B_x, B_w_r, B_w_gate, B_w_up, B_w_down, gate_w):
    def _A_ref(x, k_cache, v_cache, wq, wo):
        B, Sq, D = x.shape
        H, Dh = 32, 128
        q = (lambda x, *d: x.transpose(*d))((x @ wq).reshape(B, Sq, H, Dh), 0, 2, 1, 3)
        scores = jnp.einsum("bhqd,bhkd->bhqk", q, k_cache) * (Dh ** -0.5)
        p = _softmax(scores, axis=-1)
        o = jnp.einsum("bhqk,bhkd->bhqd", p, v_cache)
        return (lambda x, *d: x.transpose(*d))(o, 0, 2, 1, 3).reshape(B, Sq, H * Dh) @ wo

    def _B_ref(x, w_r, w_gate, w_up, w_down):
        B, S, D = x.shape
        C = 1
        r = x @ w_r
        idx = jnp.argsort(-r, axis=-1)[:, :C]
        idx_e = jnp.repeat(idx.reshape(B, C, 1), D, axis=2)
        x_sel = jnp.take_along_axis(x, idx_e, axis=1)
        g = _silu(x_sel @ w_gate)
        u = x_sel @ w_up
        y = (g * u) @ w_down
        r_sel = _sigmoid(jnp.take_along_axis(r, idx, axis=1))
        y = y * r_sel.reshape(B, C, 1)
        b_off = (jnp.arange(B) * S).reshape(B, 1)
        flat_idx = (idx + b_off).reshape(B * C)
        zero = (x * 0.0).reshape(B * S, D)
        upd = _scatter_add(zero, flat_idx, y.reshape(B * C, D), axis=0)
        return x + upd.reshape(B, S, D)

    x = A_x
    g = _sigmoid((x * gate_w).sum(-1, keepdims=True))
    a = _A_ref(x, A_k_cache, A_v_cache, A_wq, A_wo)
    b = _B_ref(x, B_w_r, B_w_gate, B_w_up, B_w_down)
    return g * a + (1 - g) * b
```

```python
import functools
import jax
import jax.numpy as jnp
from jax import lax
import jax.experimental.pallas as pl
import jax.experimental.pallas.tpu as pltpu

B, H, SK, DH, D, F = 4, 32, 8192, 128, 1024, 3584
NH = 4
ROWS = 32
NG = B * H // NH

def _make(SR=1024, DEPTH=8, compute=True, dma=True, weights=True, vmem_mb=100, wstart=(2, 4, 6), do_moe=True, wr_=8, wc_=512, wseg=4):
    G = SR // ROWS
    PER = SK // SR
    TOTAL = NG * PER
    def kernel(x_ref, k_hbm, v_hbm, wq_hbm, wo_hbm, xb_ref, wr_ref, wg_hbm, wu_hbm, wd_hbm, gw_ref,
               o_ref,
               buf, wq_v, wo_v, wg_v, wu_v, wd_v, q_s, oh_s, acc_s, b_s, m_s, l_s, o_s, sem, wsem):
        def start_stage(j, slot):
            c = j % PER; g = j // PER
            b0 = g % B; h0 = (g // B) * NH
            for t in range(G):
                for s in range(2):
                    src = (k_hbm, v_hbm)[s]
                    pltpu.make_async_copy(src.at[b0, pl.ds(h0, NH), pl.ds(c * SR + t * ROWS, ROWS)],
                                          buf.at[slot, s, :, pl.ds(t * ROWS, ROWS)], sem.at[slot]).start(priority=s)
        def wall(src, dst, si):
            if not (dma and weights): return
            ncb = src.shape[2] // wc_
            nrb = src.shape[1] // wr_
            def f(i, c):
                r = pl.multiple_of(i * wr_, wr_)
                for u in range(ncb):
                    for z in range(4 // wseg):
                      for s in range(2):
                        pltpu.make_async_copy(src.at[pl.ds(4 * s + z * wseg, wseg), pl.ds(r, wr_), pl.ds(u * wc_, wc_)],
                                              dst.at[pl.ds(4 * s + z * wseg, wseg), pl.ds(r, wr_), pl.ds(u * wc_, wc_)], wsem.at[si]).start(priority=s)
                return c
            lax.fori_loop(0, nrb, f, 0)
        def wwait(dst, si):
            if dma and weights:
                pltpu.make_async_copy(dst, dst, wsem.at[si]).wait()
        wall(wq_hbm, wq_v, 0)
        if dma:
            def f(d, c):
                start_stage(d, d)
                return c
            lax.fori_loop(0, DEPTH, f, 0)
        wall(wo_hbm, wo_v, 1)
        x = x_ref[...]
        xf = x.astype(jnp.float32)
        x8 = jnp.concatenate([xf, jnp.zeros((4, D), jnp.float32)], axis=0).astype(jnp.bfloat16)
        wwait(wq_v, 0)
        for h in range(H):
            qh = jnp.dot(x8, wq_v[:, :, h * DH:(h + 1) * DH].reshape(D, DH), preferred_element_type=jnp.float32)
            for b in range(B):
                q_s[b * (H // NH) + h // NH, pl.ds(h % NH, 1), :] = qh[b:b + 1]
        row = lax.broadcasted_iota(jnp.int32, (8, DH), 0)
        for g in range(NG):
            q_s[g, NH:8, :] = jnp.zeros((8 - NH, DH), jnp.float32)
        acc_s[...] = jnp.zeros_like(acc_s)
        oh_s[...] = jnp.zeros_like(oh_s)

        def moe():
            xb = x_ref[...].astype(jnp.float32)
            xb8 = jnp.concatenate([xb, jnp.zeros((4, D), jnp.float32)], axis=0)
            wr = wr_ref[...].astype(jnp.float32)
            t = xb8[:, 0:DH] * wr[0:1]
            for u in range(1, 8):
                t = t + xb8[:, u * DH:(u + 1) * DH] * wr[u:u + 1]
            r = jnp.sum(t, axis=-1, keepdims=True)
            xb16 = xb8.astype(jnp.bfloat16)
            wwait(wg_v, 2)
            wwait(wu_v, 3)
            wwait(wd_v, 4)
            if do_moe:
                g = jnp.dot(xb16, wg_v[...].reshape(D, F), preferred_element_type=jnp.float32)
                g = g * jax.nn.sigmoid(g)
                u = jnp.dot(xb16, wu_v[...].reshape(D, F), preferred_element_type=jnp.float32)
                y = jnp.dot((g * u).astype(jnp.bfloat16), wd_v[...].reshape(F, D), preferred_element_type=jnp.float32)
                y = y * jax.nn.sigmoid(r)
                b_s[...] = xb8 + (xb8 * 0.0 + y)
            else:
                b_s[...] = xb8

        moe_at = wstart[2] + DEPTH + 1
        rowS = lax.broadcasted_iota(jnp.int32, (8, SR), 0)

        def body(j, carry):
            slot = j % DEPTH
            c = j % PER; g = j // PER
            b = g % B; hg = g // B
            if dma:
                pltpu.make_async_copy(buf.at[slot], buf.at[slot], sem.at[slot]).wait()
            if compute:
                @pl.when(c == 0)
                def _():
                    m_s[...] = jnp.full((8, DH), -jnp.inf, jnp.float32)
                    l_s[...] = jnp.zeros((8, DH), jnp.float32)
                    o_s[...] = jnp.zeros((8, DH), jnp.float32)
                q = q_s[b * (H // NH) + hg].astype(jnp.bfloat16)
                s = None
                for i in range(NH):
                    si = lax.dot_general(q, buf[slot, 0, i], (((1,), (1,)), ((), ())), preferred_element_type=jnp.float32)
                    s = si if s is None else jnp.where(rowS == i, si, s)
                s = s * (DH ** -0.5)
                m_old = m_s[...]
                m_new = jnp.maximum(m_old, jnp.max(s, axis=-1, keepdims=True))
                alpha = jnp.exp(m_old - m_new)
                p = jnp.exp(s - m_new[:, 0:1])
                l_s[...] = alpha * l_s[...] + jnp.sum(p, axis=-1, keepdims=True)
                m_s[...] = m_new
                pb = p.astype(jnp.bfloat16)
                o = None
                for i in range(NH):
                    oi = jnp.dot(pb, buf[slot, 1, i], preferred_element_type=jnp.float32)
                    o = oi if o is None else jnp.where(row == i, oi, o)
                o_s[...] = alpha * o_s[...] + o
            if dma:
                @pl.when(j + DEPTH < TOTAL)
                def _():
                    start_stage(j + DEPTH, slot)
                for mi, (src, dst) in enumerate(((wg_hbm, wg_v), (wu_hbm, wu_v), (wd_hbm, wd_v))):
                    @pl.when(j == wstart[mi])
                    def _():
                        wall(src, dst, 2 + mi)
            if compute:
                @pl.when(c == PER - 1)
                def _():
                    on = o_s[...] / l_s[...]
                    for i in range(NH):
                        oh_s[i, pl.ds(b, 1), :] = on[i:i + 1]
                    @pl.when(b == B - 1)
                    def _():
                        @pl.when(hg == 0)
                        def _():
                            wwait(wo_v, 1)
                        a = acc_s[...]
                        for i in range(NH):
                            a = a + jnp.dot(oh_s[i].astype(jnp.bfloat16),
                                            wo_v[hg, pl.ds(i * DH, DH), :],
                                            preferred_element_type=jnp.float32)
                        acc_s[...] = a
            else:
                @pl.when(j == 4 * PER - 1)
                def _():
                    wwait(wo_v, 1)
            @pl.when(j == moe_at)
            def _():
                moe()
            return carry
        lax.fori_loop(0, TOTAL, body, 0)
        gw = gw_ref[...].astype(jnp.float32)
        t = xf[:, 0:DH] * gw[0:1]
        for u in range(1, 8):
            t = t + xf[:, u * DH:(u + 1) * DH] * gw[u:u + 1]
        g = jax.nn.sigmoid(jnp.sum(t, axis=-1, keepdims=True))
        out = g * acc_s[0:4, :] + (1.0 - g) * b_s[0:4, :]
        o_ref[...] = out.astype(o_ref.dtype)

    def fn(A_x, A_k_cache, A_v_cache, A_wq, A_wo, B_x, B_w_r, B_w_gate, B_w_up, B_w_down, gate_w):
        vm = pl.BlockSpec(memory_space=pltpu.VMEM)
        hb = pl.BlockSpec(memory_space=pl.ANY)
        r8 = lambda w: w.reshape(8, w.shape[0] // 8, w.shape[1])
        return pl.pallas_call(
            kernel,
            out_shape=jax.ShapeDtypeStruct((B, D), jnp.bfloat16),
            in_specs=[vm, hb, hb, hb, hb, vm, vm, hb, hb, hb, vm],
            out_specs=vm,
            scratch_shapes=[
                pltpu.VMEM((DEPTH, 2, NH, SR, DH), jnp.bfloat16),
                pltpu.VMEM((8, D // 8, H * DH), jnp.bfloat16),
                pltpu.VMEM((8, H * DH // 8, D), jnp.bfloat16),
                pltpu.VMEM((8, D // 8, F), jnp.bfloat16),
                pltpu.VMEM((8, D // 8, F), jnp.bfloat16),
                pltpu.VMEM((8, F // 8, D), jnp.bfloat16),
                pltpu.VMEM((NG, 8, DH), jnp.float32),
                pltpu.VMEM((NH, 8, DH), jnp.float32),
                pltpu.VMEM((8, D), jnp.float32),
                pltpu.VMEM((8, D), jnp.float32),
                pltpu.VMEM((8, DH), jnp.float32),
                pltpu.VMEM((8, DH), jnp.float32),
                pltpu.VMEM((8, DH), jnp.float32),
                pltpu.SemaphoreType.DMA((DEPTH,)),
                pltpu.SemaphoreType.DMA((5,)),
            ],
            compiler_params=pltpu.CompilerParams(vmem_limit_bytes=vmem_mb * 1024 * 1024),
        )(A_x.reshape(B, D), A_k_cache, A_v_cache, r8(A_wq), r8(A_wo), B_x.reshape(B, D), B_w_r.reshape(8, DH),
          r8(B_w_gate), r8(B_w_up), r8(B_w_down), gate_w.reshape(8, DH)).reshape(B, 1, D)
    return fn


_impl = _make()


@jax.jit
def pallas_gated_mix__mha_block_cached__moe_arch_mod__decode_kernel(
    A_x, A_k_cache, A_v_cache, A_wq, A_wo, B_x, B_w_r, B_w_gate, B_w_up, B_w_down, gate_w,
):
    return _impl(A_x, A_k_cache, A_v_cache, A_wq, A_wo, B_x, B_w_r, B_w_gate, B_w_up, B_w_down, gate_w)
```

```python
import jax
import jax.numpy as jnp
from jax import lax
import jax.experimental.pallas as pl
import jax.experimental.pallas.tpu as pltpu

B, H, SK, DH, D, F = 4, 32, 8192, 128, 1024, 3584
NH = 4
NG = B * H // NH
SR = 1024
HR = SR // 2
ROWS = 16
PER = SK // SR
TOTAL = NG * PER
DEPTH = 4
FC = 512
NL, LR = 4, 256
FE = F - NL * LR
W_START = (2, 4, 6)
FFN_AT = W_START[2] + 1 + DEPTH
NT = (((1,), (1,)), ((), ()))


def _kernel(x_hbm, k_hbm, v_hbm, wq_hbm, wo_hbm, wr_hbm, wg_hbm, wu_hbm, wd_hbm, gw_hbm,
            o_hbm,
            buf, wq_v, wo_v, wg_v, wu_v, wd_v, x_v, wr_v, gw_v, out_v,
            x8_s, h_s, q_s, oh_s, acc_s, y_s, m_s, l_s, o_s, sem, wsem, ssem):

    def start_stage(j, slot):
        c = j % PER
        g = j // PER
        r0 = ((g % B) * H + (g // B) * NH) * 2
        for t in range(HR // ROWS):
            for s, src in enumerate((k_hbm, v_hbm)):
                pltpu.make_async_copy(
                    src.at[pl.ds(r0, 2 * NH), pl.ds(c * HR + t * ROWS, ROWS)],
                    buf.at[slot, s, :, pl.ds(t * ROWS, ROWS)],
                    sem.at[slot]).start(priority=s)

    def start_weight(src, dst, si):
        def f(i, carry):
            r = pl.multiple_of(i * 8, 8)
            for u in range(src.shape[2] // 512):
                for s in range(2):
                    idx = (pl.ds(4 * s, 4), pl.ds(r, 8), pl.ds(u * 512, 512))
                    pltpu.make_async_copy(src.at[idx], dst.at[idx], wsem.at[si]).start(priority=s)
            return carry
        lax.fori_loop(0, src.shape[1] // 8, f, 0)

    def wait_all(dst, s):
        pltpu.make_async_copy(dst, dst, s).wait()

    def rows8(ref, lo, hi):
        return ref.at[lo:hi].reshape(8, (hi - lo) // 8, D)

    small = [pltpu.make_async_copy(src, dst, ssem.at[i])
             for i, (src, dst) in enumerate(((x_hbm, x_v), (wr_hbm, wr_v), (gw_hbm, gw_v)))]
    for cp in small:
        cp.start()
    start_weight(wq_hbm, wq_v, 0)

    def prime(d, carry):
        start_stage(d, d)
        return carry
    lax.fori_loop(0, DEPTH, prime, 0)
    start_weight(wo_hbm, wo_v, 1)
    for cp in small:
        cp.wait()

    x8 = jnp.concatenate([x_v[...].astype(jnp.float32), jnp.zeros((8 - B, D), jnp.float32)], axis=0)
    x8_s[...] = x8.astype(jnp.bfloat16)

    def rowdot(w_ref):
        w = w_ref[...].astype(jnp.float32)
        t = x8[:, 0:DH] * w[0:1]
        for u in range(1, 8):
            t = t + x8[:, u * DH:(u + 1) * DH] * w[u:u + 1]
        return jnp.sum(t, axis=-1, keepdims=True)

    def project_q(hg):
        col = pl.ds(pl.multiple_of(hg * NH * DH, NH * DH), NH * DH)
        qh = jnp.dot(x8_s[...], wq_v[:, :, col].reshape(D, NH * DH), preferred_element_type=jnp.float32)
        for b in range(B):
            for i in range(NH):
                q_s[hg * B + b, pl.ds(i, 1), :] = qh[b:b + 1, i * DH:(i + 1) * DH]

    q_s[...] = jnp.zeros_like(q_s)
    acc_s[...] = jnp.zeros_like(acc_s)
    oh_s[...] = jnp.zeros_like(oh_s)
    y_s[...] = jnp.zeros_like(y_s)
    wait_all(wq_v, wsem.at[0])
    project_q(0)

    row_o = lax.broadcasted_iota(jnp.int32, (8, DH), 0)
    row_s = lax.broadcasted_iota(jnp.int32, (8, SR), 0)

    def body(j, carry):
        slot = j % DEPTH
        c = j % PER
        g = j // PER
        b = g % B
        hg = g // B
        wait_all(buf.at[slot], sem.at[slot])

        @pl.when(c == 0)
        def _():
            m_s[...] = jnp.full((8, DH), -jnp.inf, jnp.float32)
            l_s[...] = jnp.zeros((8, DH), jnp.float32)
            o_s[...] = jnp.zeros((8, DH), jnp.float32)

        q = q_s[g].astype(jnp.bfloat16)
        s = None
        for i in range(NH):
            si = lax.dot_general(q, buf[slot, 0, 2 * i:2 * i + 2].reshape(SR, DH), NT,
                                 preferred_element_type=jnp.float32)
            s = si if s is None else jnp.where(row_s == i, si, s)
        s = s * (DH ** -0.5)
        m_old = m_s[...]
        m_new = jnp.maximum(m_old, jnp.max(s, axis=-1, keepdims=True))
        alpha = jnp.exp(m_old - m_new)
        p = jnp.exp(s - m_new[:, 0:1])
        l_s[...] = alpha * l_s[...] + jnp.sum(p, axis=-1, keepdims=True)
        m_s[...] = m_new
        pb = p.astype(jnp.bfloat16)
        o = None
        for i in range(NH):
            oi = jnp.dot(pb, buf[slot, 1, 2 * i:2 * i + 2].reshape(SR, DH),
                         preferred_element_type=jnp.float32)
            o = oi if o is None else jnp.where(row_o == i, oi, o)
        o_s[...] = alpha * o_s[...] + o

        @pl.when(j + DEPTH < TOTAL)
        def _():
            start_stage(j + DEPTH, slot)

        @pl.when(j + DEPTH == TOTAL)
        def _():
            for z in range(NL):
                lo = FE + z * LR
                start_weight(rows8(wd_hbm, lo, lo + LR), rows8(wd_v, lo, lo + LR), 5 + z)

        for mi, (src, dst) in enumerate(((wg_hbm, wg_v), (wu_hbm, wu_v),
                                         (rows8(wd_hbm, 0, FE), rows8(wd_v, 0, FE)))):
            @pl.when(j == W_START[mi])
            def _():
                start_weight(src, dst, 2 + mi)

        @pl.when(c == PER - 1)
        def _():
            on = o_s[...] / l_s[...]
            for i in range(NH):
                oh_s[i, pl.ds(b, 1), :] = on[i:i + 1]

            @pl.when(b == B - 1)
            def _():
                @pl.when(hg == 0)
                def _():
                    wait_all(wo_v, wsem.at[1])
                lhs = jnp.concatenate([oh_s[i] for i in range(NH)], axis=1).astype(jnp.bfloat16)
                acc_s[...] += jnp.dot(lhs, wo_v[hg], preferred_element_type=jnp.float32)

        @pl.when(j == FFN_AT)
        def _():
            wait_all(wg_v, wsem.at[2])
            wait_all(wu_v, wsem.at[3])
            wait_all(wd_v.at[0:FE], wsem.at[4])

        @pl.when(jnp.logical_and(j >= FFN_AT, j < FFN_AT + F // FC))
        def _():
            col = pl.ds(pl.multiple_of((j - FFN_AT) * FC, FC), FC)
            a = jnp.dot(x8_s[...], wg_v[:, :, col].reshape(D, FC), preferred_element_type=jnp.float32)
            u = jnp.dot(x8_s[...], wu_v[:, :, col].reshape(D, FC), preferred_element_type=jnp.float32)
            h_s[:, col] = ((a * jax.nn.sigmoid(a)) * u).astype(jnp.bfloat16)

        @pl.when(jnp.logical_and(j >= FFN_AT + F // FC, j < FFN_AT + F // FC + FE // FC))
        def _():
            col = pl.ds(pl.multiple_of((j - FFN_AT - F // FC) * FC, FC), FC)
            y_s[...] += jnp.dot(h_s[:, col], wd_v[col, :], preferred_element_type=jnp.float32)

        @pl.when(jnp.logical_and(j % (B * PER) == 1, hg + 1 < H // NH))
        def _():
            project_q(hg + 1)

        return carry

    lax.fori_loop(0, TOTAL, body, 0)

    gate = jax.nn.sigmoid(rowdot(gw_v))
    r_sel = jax.nn.sigmoid(rowdot(wr_v))
    ga = gate * acc_s[...]
    y = y_s[...]
    for z in range(NL):
        lo = FE + z * LR
        wait_all(wd_v.at[lo:lo + LR], wsem.at[5 + z])
        y = y + jnp.dot(h_s[:, lo:lo + LR], wd_v[lo:lo + LR, :], preferred_element_type=jnp.float32)
    y = y * r_sel
    out = ga + (1.0 - gate) * (x8 + (x8 * 0.0 + y))
    out_v[...] = out[0:B].astype(out_v.dtype)
    cp = pltpu.make_async_copy(out_v, o_hbm, ssem.at[0])
    cp.start()
    cp.wait()


@jax.jit
def pallas_gated_mix__mha_block_cached__moe_arch_mod__decode_kernel(
    A_x, A_k_cache, A_v_cache, A_wq, A_wo, B_x, B_w_r, B_w_gate, B_w_up, B_w_down, gate_w,
):
    del B_x
    hbm = pl.BlockSpec(memory_space=pl.ANY)
    split8 = lambda w: w.reshape(8, w.shape[0] // 8, w.shape[1])
    halves = lambda c: c.reshape(B * H * 2, SK // 2, DH)
    out = pl.pallas_call(
        _kernel,
        out_shape=jax.ShapeDtypeStruct((B, D), A_x.dtype),
        in_specs=[hbm] * 10,
        out_specs=hbm,
        scratch_shapes=[
            pltpu.VMEM((DEPTH, 2, 2 * NH, HR, DH), jnp.bfloat16),
            pltpu.VMEM((8, D // 8, H * DH), jnp.bfloat16),
            pltpu.VMEM((8, H * DH // 8, D), jnp.bfloat16),
            pltpu.VMEM((8, D // 8, F), jnp.bfloat16),
            pltpu.VMEM((8, D // 8, F), jnp.bfloat16),
            pltpu.VMEM((F, D), jnp.bfloat16),
            pltpu.VMEM((B, D), jnp.bfloat16),
            pltpu.VMEM((8, DH), jnp.bfloat16),
            pltpu.VMEM((8, DH), jnp.bfloat16),
            pltpu.VMEM((B, D), A_x.dtype),
            pltpu.VMEM((8, D), jnp.bfloat16),
            pltpu.VMEM((8, F), jnp.bfloat16),
            pltpu.VMEM((NG, 8, DH), jnp.float32),
            pltpu.VMEM((NH, 8, DH), jnp.float32),
            pltpu.VMEM((8, D), jnp.float32),
            pltpu.VMEM((8, D), jnp.float32),
            pltpu.VMEM((8, DH), jnp.float32),
            pltpu.VMEM((8, DH), jnp.float32),
            pltpu.VMEM((8, DH), jnp.float32),
            pltpu.SemaphoreType.DMA((DEPTH,)),
            pltpu.SemaphoreType.DMA((5 + NL,)),
            pltpu.SemaphoreType.DMA((3,)),
        ],
        compiler_params=pltpu.CompilerParams(vmem_limit_bytes=100 * 1024 * 1024),
    )(A_x.reshape(B, D), halves(A_k_cache), halves(A_v_cache), split8(A_wq), split8(A_wo),
      B_w_r.reshape(8, DH), split8(B_w_gate), split8(B_w_up), B_w_down, gate_w.reshape(8, DH))
    return out.reshape(B, 1, D)
```
